```python
import jax
import jax.numpy as jnp

def _softmax(x, axis=-1):
    return jax.nn.softmax(x, axis=axis)
def _gelu(x):
    return jax.nn.gelu(x, approximate=True)
def _silu(x):
    return jax.nn.silu(x)
def _sigmoid(x):
    return jax.nn.sigmoid(x)
def _layernorm(x, axis=-1, eps=1e-5):
    m = jnp.mean(x, axis=axis, keepdims=True)
    v = jnp.var(x, axis=axis, keepdims=True)
    return (x - m) / jnp.sqrt(v + eps)
def _scatter_add(tgt, idx, src, axis=0):
    return tgt.at[idx].add(src)
def _segment_sum(src, seg, n):
    return jax.ops.segment_sum(src, seg, n)
class _Rng:
    def __init__(self, key):
        self._k = key
    def _next(self):
        self._k, sub = jax.random.split(self._k)
        return sub
    def normal(self, shape):
        return jax.random.normal(self._next(), shape, dtype=jnp.bfloat16)
    def randint(self, lo, hi, shape):
        return jax.random.randint(self._next(), shape, lo, hi, dtype=jnp.int32)
    def uniform(self, shape, lo=0.0, hi=1.0):
        return jax.random.uniform(self._next(), shape, jnp.bfloat16, lo, hi)
    def permutation(self, n):
        return jax.random.permutation(self._next(), n)


kernel_name = 'interleave_layers__sliding_block_cached__dense_activation_gelu__decode'

def _fwd_setup_inputs():
    _rng = _Rng(jax.random.key(int.from_bytes(__import__("os").urandom(4), "little")))
    _w = (lambda a: (lambda t: t.astype(jnp.bfloat16) if jnp.issubdtype(t.dtype, jnp.floating) else t)(jnp.asarray(a)))
    def _A_setup():
        B, Sq, D = 2, 1, 512
        Hq, Hkv, Sk, Dh = 32, 8, 32768, 128
        assert Hq % Hkv == 0, (Hq, Hkv)
        return {
            "x": _w((lambda *s: _rng.normal(s) * 0.05)(B, Sq, D)),
            "k_cache": _w((lambda *s: _rng.normal(s) * 0.05)(B, Hkv, Sk, Dh)),
            "v_cache": _w((lambda *s: _rng.normal(s) * 0.05)(B, Hkv, Sk, Dh)),
            "wq": _w((lambda *s: _rng.normal(s) * 0.05)(D, Hq * Dh) * (D ** -0.5)),
            "wo": _w((lambda *s: _rng.normal(s) * 0.05)(Hq * Dh, D) * ((Hq * Dh) ** -0.5)),
        }
    _A_in = _A_setup()

    def _B_setup():
        B, S, D, F = 2, 1, 512, 1792
        return {
            "x": _w((lambda *s: _rng.normal(s) * 0.05)(B, S, D)),
            "w1": _w((lambda *s: _rng.normal(s) * 0.05)(D, F) * (D ** -0.5)),
            "b1": _w((lambda *s: _rng.normal(s) * 0.05)(F) * 0.01),
            "w2": _w((lambda *s: _rng.normal(s) * 0.05)(F, D) * (F ** -0.5)),
            "b2": _w((lambda *s: _rng.normal(s) * 0.05)(D) * 0.01),
        }
    _B_in = _B_setup()

    return {
        "A_x": _A_in["x"],
        "A_k_cache": _A_in["k_cache"],
        "A_v_cache": _A_in["v_cache"],
        "A_wq": _A_in["wq"],
        "A_wo": _A_in["wo"],
        "B_x": _B_in["x"],
        "B_w1": _B_in["w1"],
        "B_b1": _B_in["b1"],
        "B_w2": _B_in["w2"],
        "B_b2": _B_in["b2"],
    }

def _fwd_reference(A_x, A_k_cache, A_v_cache, A_wq, A_wo, B_x, B_w1, B_b1, B_w2, B_b2):
    def _A_ref(x, k_cache, v_cache, wq, wo):
        B, Sq, D = x.shape
        Hq, Dh = 32, 128
        Hkv, Sk = k_cache.shape[1], k_cache.shape[2]
        W = min(4096, max(256, Sk // 4))
        rep = Hq // Hkv
        q = (lambda x, *d: x.transpose(*d))((x @ wq).reshape(B, Sq, Hq, Dh), 0, 2, 1, 3)
        k = jnp.repeat(k_cache[:, :, Sk - W:, :], rep, axis=1)
        v = jnp.repeat(v_cache[:, :, Sk - W:, :], rep, axis=1)
        scores = jnp.einsum("bhqd,bhkd->bhqk", q, k) * (Dh ** -0.5)
        p = _softmax(scores, axis=-1)
        o = jnp.einsum("bhqk,bhkd->bhqd", p, v)
        return (lambda x, *d: x.transpose(*d))(o, 0, 2, 1, 3).reshape(B, Sq, Hq * Dh) @ wo

    def _B_ref(x, w1, b1, w2, b2):
        h = jnp.einsum("bsd,df->bsf", x, w1) + b1
        h = _gelu(h)
        return jnp.einsum("bsf,fd->bsd", h, w2) + b2

    x = A_x
    x = x + _A_ref(_layernorm(x, axis=-1), A_k_cache, A_v_cache, A_wq, A_wo)
    x = x + _B_ref(_layernorm(x, axis=-1), B_w1, B_b1, B_w2, B_b2)
    x = x + _A_ref(_layernorm(x, axis=-1), A_k_cache, A_v_cache, A_wq, A_wo)
    x = x + _B_ref(_layernorm(x, axis=-1), B_w1, B_b1, B_w2, B_b2)
    return x


def setup_inputs():
    _inp = _fwd_setup_inputs()
    _gk = jax.random.fold_in(jax.random.key(int.from_bytes(__import__("os").urandom(4), "little")), 2**31 - 1)
    _shapes = [[2, 1, 512]]
    _dtypes = ['bfloat16']
    _gks = jax.random.split(_gk, len(_shapes))
    _gs = [jax.random.normal(k, s, dtype=jnp.dtype(d)) * 0.05 for k, s, d in zip(_gks, _shapes, _dtypes)]
    _inp["grad_out"] = _gs[0]
    return _inp

def reference(A_x, A_k_cache, A_v_cache, A_wq, A_wo, B_w1, B_b1, B_w2, B_b2, B_x, grad_out):
    _const = dict(B_x=B_x)
    def _f(*_d):
        return _fwd_reference(**{'A_x': _d[0], 'A_k_cache': _d[1], 'A_v_cache': _d[2], 'A_wq': _d[3], 'A_wo': _d[4], 'B_w1': _d[5], 'B_b1': _d[6], 'B_w2': _d[7], 'B_b2': _d[8], **_const})
    _out, _vjp = jax.vjp(_f, A_x, A_k_cache, A_v_cache, A_wq, A_wo, B_w1, B_b1, B_w2, B_b2)
    _grads = _vjp(grad_out)
    _out0 = jnp.asarray(_out)
    return (_out0, *[jnp.asarray(_g) for _g in _grads])
```

```python
import math

import jax
import jax.numpy as jnp
from jax import lax
from jax.experimental import pallas as pl
from jax.experimental.pallas import tpu as pltpu

_HQ = 32
_EPS = 1e-5
_GELU_C = math.sqrt(2.0 / math.pi)
_GELU_A = 0.044715

_F32 = jnp.float32
_BF16 = jnp.bfloat16

_NN = (((1,), (0,)), ((), ()))
_NT = (((1,), (1,)), ((), ()))
_TN = (((0,), (0,)), ((), ()))

CFG = dict(zseg=8, zrows=128, zero=True, f0=40, s0=12, f=16, s=12, sw=8, dw='q4')


def _dot(a, b, dims=_NN):
    return lax.dot_general(a.astype(_BF16), b.astype(_BF16), dims,
                           preferred_element_type=_F32)


def _layernorm(x):
    mu = jnp.mean(x, axis=-1, keepdims=True)
    xc = x - mu
    var = jnp.mean(xc * xc, axis=-1, keepdims=True)
    rstd = 1.0 / jnp.sqrt(var + _EPS)
    return xc * rstd, rstd


def _layernorm_bwd(dy, y, rstd):
    return rstd * (dy - jnp.mean(dy, axis=-1, keepdims=True)
                   - y * jnp.mean(dy * y, axis=-1, keepdims=True))


def _kernel(x_hbm, k_hbm, v_hbm, wq_hbm, wo_hbm, w1_hbm, b1_hbm, w2_hbm, b2_hbm, g_hbm,
            out_hbm, dx_hbm, dk_hbm, dv_hbm, dwq_hbm, dwo_hbm, dw1_hbm, db1_hbm,
            dw2_hbm, db2_hbm,
            kb, vb, wqb, wob, w1b, w2b, xb, gb, b1b, b2b, zb,
            p_all, ds_all, q_all, do_all, t_all, pt, dst,
            dkb, dvb, dwqb, dwob, dw1b, dw2b, outb, dxb, db1b, db2b,
            in_sem, out_sem):
    _ZSEG = CFG['zseg']; _ZROWS = CFG['zrows']
    nb, hkv, win, dh = kb.shape
    sk = k_hbm.shape[2]
    d_model = wqb.shape[0]
    rep = _HQ // hkv
    zero_rows = sk - win
    scale = dh ** -0.5
    nslab = nb * hkv
    lrows = hkv * 8

    window_rows = pl.ds(zero_rows, win)
    reads = [pltpu.make_async_copy(s, d, in_sem.at[0]) for s, d in (
        (k_hbm.at[:, :, window_rows, :], kb), (v_hbm.at[:, :, window_rows, :], vb),
        (wq_hbm, wqb), (wo_hbm, wob), (w1_hbm, w1b), (w2_hbm, w2b),
        (x_hbm, xb), (g_hbm, gb), (b1_hbm, b1b), (b2_hbm, b2b))]
    for c in reads:
        c.start()

    zb[...] = jnp.zeros(zb.shape, zb.dtype)
    chunks = zero_rows // _ZROWS
    per_array = nb * chunks

    def zero_fill(which, start, count):
        dst_ref = (dk_hbm, dv_hbm)[which]
        if not CFG['zero'] or (isinstance(count, int) and count == 0):
            return

        def body(i, carry):
            b = i // chunks
            row = pl.multiple_of((i - b * chunks) * _ZROWS, _ZROWS)
            pltpu.make_async_copy(
                zb, dst_ref.at[b, :, pl.ds(row, _ZROWS), :], out_sem.at[which]).start()
            return carry

        lax.fori_loop(start, start + count, body, 0)

    issued = [0, 0]

    def reserve(count):
        which = 0 if issued[0] + count <= per_array else 1
        base = issued[which]
        issued[which] += count
        assert issued[which] <= per_array
        return which, base

    def fill(count):
        which, base = reserve(count)
        zero_fill(which, base, count)

    def loop_fill(count):
        which, base = reserve(count * hkv)
        return lambda g: zero_fill(which, base + g * count, count)

    row = lax.broadcasted_iota(jnp.int32, (8, 1), 0)
    first_batch = row < rep
    head_of_row = row % rep

    def replicate(ref):
        v = ref[...].astype(_F32)
        return jnp.where(first_batch, v[0:1], v[1:2])

    def compact(v, dtype):
        two = lax.broadcasted_iota(jnp.int32, (nb, 1), 0)
        return jnp.where(two == 0, v[0:1], v[rep:rep + 1]).astype(dtype)

    def per_batch(a0, a1):
        return jnp.where(first_batch, a0, a1)

    def batch_sum(v):
        s0 = jnp.sum(jnp.where(first_batch, v, 0.0), axis=0, keepdims=True)
        s1 = jnp.sum(jnp.where(first_batch, 0.0, v), axis=0, keepdims=True)
        return per_batch(s0, s1)

    def split_heads(full, dst_ref, base):
        for g in range(hkv):
            t = full[:, g * rep * dh:(g * rep + 1) * dh]
            for r in range(1, rep):
                h = g * rep + r
                t = jnp.where(head_of_row == r, full[:, h * dh:(h + 1) * dh], t)
            dst_ref[pl.ds(base + g * 8, 8), :] = t

    def merge_heads(src_ref):
        parts = []
        for g in range(hkv):
            t = src_ref[pl.ds(g * 8, 8), :]
            parts += [jnp.where(head_of_row == r, t, 0.0) for r in range(rep)]
        return jnp.concatenate(parts, axis=1)

    def once(v):
        return jnp.where(head_of_row == 0, v, 0.0)

    def tile(layer, g):
        return pl.ds(pl.multiple_of(layer * lrows + g * 8, 8), 8)

    def attn_fwd(layer, x, per_step):
        xn, rstd = _layernorm(x)
        split_heads(_dot(xn, wqb[...]), q_all, layer * lrows)
        step_fill = loop_fill(per_step)

        def body(g, carry):
            q = q_all[tile(layer, g), :]
            s = per_batch(_dot(q, kb[0, g], _NT), _dot(q, kb[1, g], _NT)) * scale
            e = jnp.exp(s - jnp.max(s, axis=-1, keepdims=True))
            p = e / jnp.sum(e, axis=-1, keepdims=True)
            p_all[tile(layer, g), :] = p
            t_all[tile(0, g), :] = per_batch(_dot(p, vb[0, g]), _dot(p, vb[1, g]))
            step_fill(g)
            return carry

        lax.fori_loop(0, hkv, body, 0)
        o = merge_heads(t_all)
        return x + batch_sum(_dot(o, wob[...])), (xn, rstd, o)

    def ffn_fwd(x, b1, b2):
        xn, rstd = _layernorm(x)
        h = _dot(xn, w1b[...]) + b1
        t = jnp.tanh(_GELU_C * (h + _GELU_A * h * h * h))
        a = 0.5 * h * (1.0 + t)
        return x + _dot(a, w2b[...]) + b2, (xn, rstd, h, t, a)

    def ffn_bwd(dy, saved):
        xn, rstd, h, t, _ = saved
        da = _dot(dy, w2b[...], _NT)
        dgelu = 0.5 * (1.0 + t) + (0.5 * _GELU_C) * h * (1.0 - t * t) * (
            1.0 + (3.0 * _GELU_A) * h * h)
        dh_ = da * dgelu
        return dy + _layernorm_bwd(_dot(dh_, w1b[...], _NT), xn, rstd), dh_

    def attn_bwd(layer, dy, saved, per_step):
        xn, rstd, _ = saved
        split_heads(_dot(dy, wob[...], _NT), do_all, layer * lrows)
        step_fill = loop_fill(per_step)

        def body(g, carry):
            do = do_all[tile(layer, g), :]
            dp = per_batch(_dot(do, vb[0, g], _NT), _dot(do, vb[1, g], _NT))
            p = p_all[tile(layer, g), :]
            ds = p * (dp - jnp.sum(dp * p, axis=-1, keepdims=True)) * scale
            ds_all[tile(layer, g), :] = ds
            t_all[tile(0, g), :] = per_batch(_dot(ds, kb[0, g]), _dot(ds, kb[1, g]))
            step_fill(g)
            return carry

        lax.fori_loop(0, hkv, body, 0)
        dq = merge_heads(t_all)
        return dy + _layernorm_bwd(batch_sum(_dot(dq, wqb[...], _NT)), xn, rstd), dq

    for c in reads:
        c.wait()
    fill(CFG['f0'])
    x0 = replicate(xb)
    x1, att_a = attn_fwd(0, x0, CFG['s0'])
    fill(CFG['f'])
    b1 = b1b[...].astype(_F32).reshape(1, -1)
    b2 = b2b[...].astype(_F32).reshape(1, -1)
    x2, ffn_a = ffn_fwd(x1, b1, b2)
    fill(CFG['f'])
    x3, att_b = attn_fwd(1, x2, CFG['s'])
    fill(CFG['f'])
    x4, ffn_b = ffn_fwd(x3, b1, b2)
    outb[...] = compact(x4, outb.dtype)
    cp_out = pltpu.make_async_copy(outb, out_hbm, out_sem.at[2])
    cp_out.start()

    g4 = replicate(gb)
    g3, dh_b = ffn_bwd(g4, ffn_b)
    fill(CFG['f'])
    g2, dq_b = attn_bwd(1, g3, att_b, CFG['s'])
    fill(CFG['f'])
    g1, dh_a = ffn_bwd(g2, ffn_a)
    fill(CFG['f'])
    g0, dq_a = attn_bwd(0, g1, att_a, CFG['s'])
    dxb[...] = compact(g0, dxb.dtype)
    cp_dx = pltpu.make_async_copy(dxb, dx_hbm, out_sem.at[3])
    cp_dx.start()
    fill(CFG['f'])

    def stack(a, b):
        return jnp.concatenate([a, b], axis=0)

    dy_ffn = stack(once(g2), once(g4))
    dh_ffn = stack(once(dh_a), once(dh_b))
    db1b[...] = jnp.sum(dh_ffn, axis=0).astype(db1b.dtype)
    db2b[...] = jnp.sum(dy_ffn, axis=0).astype(db2b.dtype)
    def outer(dst_ref, a, b):
        at = a.T.astype(_BF16)
        b = b.astype(_BF16)
        rows = dst_ref.shape[1]
        for i in range(dst_ref.shape[0]):
            dst_ref[i] = _dot(at[i * rows:(i + 1) * rows], b).astype(dst_ref.dtype)

    outer(dw1b, stack(ffn_a[0], ffn_b[0]), dh_ffn)
    outer(dw2b, stack(ffn_a[4], ffn_b[4]), dy_ffn)
    fill(CFG['f'])
    outer(dwqb, stack(att_a[0], att_b[0]), stack(dq_a, dq_b))
    fill(CFG['f'])
    outer(dwob, stack(att_a[2], att_b[2]), stack(g1, g3))
    small_out = [pltpu.make_async_copy(s, d, out_sem.at[4 + i]) for i, (s, d) in enumerate(
        [(db1b, db1_hbm), (db2b, db2_hbm), (dw1b, dw1_hbm), (dw2b, dw2_hbm),
         (dwqb, dwq_hbm), (dwob, dwo_hbm)])]
    if CFG['dw'] == 'big':
        for c in small_out:
            c.start()
    else:
        for c in small_out[:2]:
            c.start()

        def spread(s3, d3, sem, rows, cols):
            _, n, m = s3.shape
            ncol = m // cols
            assert m % cols == 0 and n % rows == 0

            def body(i, carry):
                r = pl.multiple_of((i // ncol) * rows, rows)
                c = pl.multiple_of((i % ncol) * cols, 128)
                idx = (slice(None), pl.ds(r, rows), pl.ds(c, cols))
                pltpu.make_async_copy(s3.at[idx], d3.at[idx], sem).start()
                return carry
            lax.fori_loop(0, (n // rows) * ncol, body, 0)
        spread(dw1b, dw1_hbm, out_sem.at[6], 16, 896)
        spread(dw2b, dw2_hbm, out_sem.at[7], 32, 512)
        spread(dwqb, dwq_hbm, out_sem.at[8], 16, 1024)
        spread(dwob, dwo_hbm, out_sem.at[9], 32, 512)

    pt[...] = p_all[...].T.astype(pt.dtype)
    dst[...] = ds_all[...].T.astype(dst.dtype)
    stack_row = lax.broadcasted_iota(jnp.int32, (2 * lrows, 1), 0)
    step_fill = loop_fill(CFG['sw'])

    def window_body(g, carry):
        for b in range(nb):
            mine = (stack_row % lrows) // rep == g * nb + b
            dkb[b, g] = _dot(dst[...], jnp.where(mine, q_all[...], 0.0)).astype(dkb.dtype)
            dvb[b, g] = _dot(pt[...], jnp.where(mine, do_all[...], 0.0)).astype(dvb.dtype)
        step_fill(g)
        return carry

    lax.fori_loop(0, hkv, window_body, 0)

    for which, (src, dst_ref) in enumerate(((dkb, dk_hbm), (dvb, dv_hbm))):
        for b in range(nb):
            def body(i, carry, src=src, dst_ref=dst_ref, b=b, which=which):
                r0 = pl.multiple_of(i * _ZROWS, _ZROWS)
                pltpu.make_async_copy(
                    src.at[b, :, pl.ds(r0, _ZROWS), :],
                    dst_ref.at[b, :, pl.ds(zero_rows + r0, _ZROWS), :],
                    out_sem.at[which]).start()
                return carry

            lax.fori_loop(0, win // _ZROWS, body, 0)

    for which in range(2):
        zero_fill(which, issued[which], per_array - issued[which])

    if CFG['zero']:
        pltpu.make_async_copy(dk_hbm, dk_hbm, out_sem.at[0]).wait()
        pltpu.make_async_copy(dv_hbm, dv_hbm, out_sem.at[1]).wait()
    else:
        pltpu.make_async_copy(dkb, dkb, out_sem.at[0]).wait()
        pltpu.make_async_copy(dvb, dvb, out_sem.at[1]).wait()
    for c in [cp_out, cp_dx] + small_out:
        c.wait()


@jax.jit
def pallas_interleave_layers__sliding_block_cached__dense_activation_gelu__decode_kernel(
    A_x: jax.Array,
    A_k_cache: jax.Array,
    A_v_cache: jax.Array,
    A_wq: jax.Array,
    A_wo: jax.Array,
    B_x: jax.Array,
    B_w1: jax.Array,
    B_b1: jax.Array,
    B_w2: jax.Array,
    B_b2: jax.Array,
    grad_out: jax.Array,
):
    _ZSEG = CFG['zseg']; _ZROWS = CFG['zrows']
    nb, hkv, sk, dh = A_k_cache.shape
    win = min(4096, max(256, sk // 4))
    assert nb == 2 and _HQ // hkv == 4 and A_x.shape[1] == 1
    assert (sk - win) % _ZROWS == 0 and win % _ZROWS == 0 and (nb * hkv) % _ZSEG == 0

    def like(a):
        return jax.ShapeDtypeStruct(a.shape, a.dtype)

    def vmem(a):
        return pltpu.VMEM(a.shape, a.dtype)

    x_shape = A_x.shape
    A_x = A_x.reshape(nb, -1)
    grad_out = grad_out.reshape(nb, -1)
    window = pltpu.VMEM((nb, hkv, win, dh), A_k_cache.dtype)
    stack_rows = 2 * hkv * 8
    inputs = (A_x, A_k_cache, A_v_cache, A_wq, A_wo, B_w1, B_b1, B_w2, B_b2, grad_out)

    def blocks(w):
        return jax.ShapeDtypeStruct((4, w.shape[0] // 4, w.shape[1]), w.dtype)

    d_wq, d_wo, d_w1, d_w2 = blocks(A_wq), blocks(A_wo), blocks(B_w1), blocks(B_w2)
    outputs = (grad_out, A_x, A_k_cache, A_v_cache, d_wq, d_wo, d_w1, B_b1, d_w2, B_b2)
    any_spec = pl.BlockSpec(memory_space=pl.ANY)
    out, dx, dk, dv, dwq, dwo, dw1, db1, dw2, db2 = pl.pallas_call(
        _kernel,
        out_shape=[like(a) for a in outputs],
        in_specs=[any_spec] * len(inputs),
        out_specs=[any_spec] * len(outputs),
        scratch_shapes=[
            window, window, vmem(A_wq), vmem(A_wo), vmem(B_w1), vmem(B_w2),
            vmem(A_x), vmem(grad_out), vmem(B_b1), vmem(B_b2),
            pltpu.VMEM((hkv, _ZROWS, dh), A_k_cache.dtype),
            pltpu.VMEM((stack_rows, win), _F32), pltpu.VMEM((stack_rows, win), _F32),
            pltpu.VMEM((stack_rows, dh), _F32), pltpu.VMEM((stack_rows, dh), _F32),
            pltpu.VMEM((stack_rows // 2, dh), _F32),
            pltpu.VMEM((win, stack_rows), _BF16), pltpu.VMEM((win, stack_rows), _BF16),
            window, window, vmem(d_wq), vmem(d_wo), vmem(d_w1), vmem(d_w2),
            vmem(grad_out), vmem(A_x), vmem(B_b1), vmem(B_b2),
            pltpu.SemaphoreType.DMA((1,)),
            pltpu.SemaphoreType.DMA((10,)),
        ],
        compiler_params=pltpu.CompilerParams(vmem_limit_bytes=110 * 1024 * 1024),
    )(*inputs)
    return (out.reshape(x_shape), dx.reshape(x_shape), dk, dv,
            dwq.reshape(A_wq.shape), dwo.reshape(A_wo.shape), dw1.reshape(B_w1.shape), db1,
            dw2.reshape(B_w2.shape), db2)
```

```python
import math

import jax
import jax.numpy as jnp
from jax import lax
from jax.experimental import pallas as pl
from jax.experimental.pallas import tpu as pltpu

_HQ = 32
_LAYERS = 2
_EPS = 1e-5
_GELU_C = math.sqrt(2.0 / math.pi)
_GELU_A = 0.044715

_F32 = jnp.float32
_BF16 = jnp.bfloat16
_NN = (((1,), (0,)), ((), ()))
_NT = (((1,), (1,)), ((), ()))

_ZERO_ROWS = 64
_WINDOW_ROWS = 16
_WEIGHT_ROWS = 16
_LATE_ROWS = 64


def _dot(a, b, dims=_NN):
    return lax.dot_general(a.astype(_BF16), b.astype(_BF16), dims,
                           preferred_element_type=_F32)


def _layernorm(x):
    xc = x - jnp.mean(x, axis=-1, keepdims=True)
    rstd = 1.0 / jnp.sqrt(jnp.mean(xc * xc, axis=-1, keepdims=True) + _EPS)
    return xc * rstd, rstd


def _layernorm_bwd(dy, y, rstd):
    return rstd * (dy - jnp.mean(dy, axis=-1, keepdims=True)
                   - y * jnp.mean(dy * y, axis=-1, keepdims=True))


def _gelu_tanh(h):
    return jnp.tanh(_GELU_C * (h + _GELU_A * h * h * h))


def _gelu(h):
    return 0.5 * h * (1.0 + _gelu_tanh(h))


def _gelu_grad(h):
    t = _gelu_tanh(h)
    return 0.5 * (1.0 + t) + (0.5 * _GELU_C) * h * (1.0 - t * t) * (
        1.0 + (3.0 * _GELU_A) * h * h)


def _kernel(x_hbm, k_hbm, v_hbm, wq_hbm, wo_hbm, w1_hbm, b1_hbm, w2_hbm, b2_hbm, g_hbm,
            out_hbm, dx_hbm, dk_hbm, dv_hbm, dwq_hbm, dwo_hbm, dw1_hbm, db1_hbm,
            dw2_hbm, db2_hbm,
            k_buf, v_buf, wq, wo, w1, w2, x_buf, g_buf, b1, b2, zeros,
            p_all, ds_all, q_all, o_all, do_all, dq_all,
            att_xn, att_rstd, att_dy, ffn_xn, ffn_rstd, ffn_dy, ffn_h, ffn_dh,
            p_t, ds_t, att_xn_t,
            dk_buf, dv_buf, dwq, dwo, dw1, dw2, out_buf, dx_buf, db1, db2,
            in_sem, out_sem):
    nb, hkv, win, dh = k_buf.shape
    sk = k_hbm.shape[2]
    rep = _HQ // hkv
    group_cols = rep * dh
    layer_rows = hkv * 8
    scale = dh ** -0.5

    early_rows = win - _LATE_ROWS
    reads = [pltpu.make_async_copy(s, d, in_sem.at[0]) for s, d in (
        (wq_hbm, wq), (x_hbm, x_buf), (g_hbm, g_buf), (b1_hbm, b1), (b2_hbm, b2),
        (wo_hbm, wo), (w1_hbm, w1), (w2_hbm, w2),
        (k_hbm.at[:, :, pl.ds(sk - win, win), :], k_buf),
        (v_hbm.at[:, :, pl.ds(sk - win, early_rows), :],
         v_buf.at[:, :, pl.ds(0, early_rows), :]))]
    last_read = pltpu.make_async_copy(
        v_hbm.at[:, :, pl.ds(sk - _LATE_ROWS, _LATE_ROWS), :],
        v_buf.at[:, :, pl.ds(early_rows, _LATE_ROWS), :], in_sem.at[1])
    for c in reads:
        c.start()
    last_read.start()

    zeros[...] = jnp.zeros(zeros.shape, zeros.dtype)
    cache_grads = (dk_hbm, dv_hbm)
    zero_segs = dk_hbm.shape[1] - 1
    per_slab = win // _ZERO_ROWS
    num_zero = nb * hkv * per_slab
    per_pass = hkv + 2
    lead = num_zero // 16
    batch = (num_zero - lead) // (2 * _LAYERS * per_pass)

    def zero_fill(which, start, count):
        def body(i, carry):
            r = pl.multiple_of(lax.rem(i, per_slab) * _ZERO_ROWS, _ZERO_ROWS)
            pltpu.make_async_copy(
                zeros,
                cache_grads[which].at[lax.div(i, per_slab), pl.ds(0, zero_segs),
                                      pl.ds(r, _ZERO_ROWS), :],
                out_sem.at[which]).start()
            return carry

        lax.fori_loop(start, start + count, body, 0)

    def dk_batch(t):
        zero_fill(0, lead + t * batch, batch)

    def dv_batch(t):
        zero_fill(1, t * batch, batch)

    first_batch = lax.broadcasted_iota(jnp.int32, (8, 1), 0) < rep

    def head_of_row(t):
        return lax.broadcasted_iota(jnp.int32, (t.shape[0], 1), 0) % rep

    def per_batch(a0, a1):
        return jnp.where(first_batch, a0, a1)

    def replicate(ref):
        v = ref[...].astype(_F32)
        return per_batch(v[0:1], v[1:2])

    def compact(v):
        b = lax.broadcasted_iota(jnp.int32, (nb, 1), 0)
        return jnp.where(b == 0, v[0:1], v[rep:rep + 1])

    def batch_sum(v):
        return per_batch(jnp.sum(per_batch(v, 0.0), axis=0, keepdims=True),
                         jnp.sum(per_batch(0.0, v), axis=0, keepdims=True))

    def pick_heads(full):
        h = head_of_row(full)
        t = full[:, :dh]
        for r in range(1, rep):
            t = jnp.where(h == r, full[:, r * dh:(r + 1) * dh], t)
        return t

    def spread_heads(t):
        h = head_of_row(t)
        return jnp.concatenate([jnp.where(h == r, t, 0.0) for r in range(rep)], axis=1)

    def one_replica(t):
        return jnp.where(head_of_row(t) == 0, t, 0.0)

    def head_tile(layer, g):
        return pl.ds(pl.multiple_of(layer * layer_rows + g * 8, 8), 8)

    def layer_tile(layer):
        return pl.ds(pl.multiple_of(layer * 8, 8), 8)

    def head_cols(g):
        return pl.ds(pl.multiple_of(g * group_cols, group_cols), group_cols)

    def forward(layer, x):
        t0 = layer * per_pass
        rows = layer_tile(layer)
        xn, rstd = _layernorm(x)
        att_xn[rows, :] = xn
        att_rstd[rows, :] = jnp.broadcast_to(rstd, (8, att_rstd.shape[1]))

        def head(g, acc):
            q = pick_heads(_dot(xn, wq[:, head_cols(g)]))
            s = per_batch(_dot(q, k_buf[0, g], _NT), _dot(q, k_buf[1, g], _NT)) * scale
            e = jnp.exp(s - jnp.max(s, axis=-1, keepdims=True))
            p = e / jnp.sum(e, axis=-1, keepdims=True)
            o = per_batch(_dot(p, v_buf[0, g]), _dot(p, v_buf[1, g]))
            q_all[head_tile(layer, g), :] = q
            p_all[head_tile(layer, g), :] = p
            o_all[head_tile(layer, g), :] = o
            acc = acc + _dot(spread_heads(o), wo[head_cols(g), :])
            dk_batch(t0 + g)
            return acc

        x = x + batch_sum(lax.fori_loop(0, hkv, head, jnp.zeros_like(x)))

        xn2, rstd2 = _layernorm(x)
        h = _dot(xn2, w1[...]) + b1[...].astype(_F32).reshape(1, -1)
        ffn_xn[rows, :] = xn2
        ffn_rstd[rows, :] = jnp.broadcast_to(rstd2, (8, ffn_rstd.shape[1]))
        ffn_h[rows, :] = h
        a = _gelu(h)
        dk_batch(t0 + hkv)
        x = x + _dot(a, w2[...]) + b2[...].astype(_F32).reshape(1, -1)
        dk_batch(t0 + hkv + 1)
        return x

    def backward(step, dy):
        layer = _LAYERS - 1 - step
        t0 = (_LAYERS + step) * per_pass
        rows = layer_tile(layer)
        ffn_dy[rows, :] = dy
        d_h = _dot(dy, w2[...], _NT) * _gelu_grad(ffn_h[rows, :])
        ffn_dh[rows, :] = d_h
        dk_batch(t0)
        dy = dy + _layernorm_bwd(_dot(d_h, w1[...], _NT), ffn_xn[rows, :],
                                 ffn_rstd[rows, :1])
        att_dy[rows, :] = dy
        dk_batch(t0 + 1)

        def head(g, acc):
            do = pick_heads(_dot(dy, wo[head_cols(g), :], _NT))
            dp = per_batch(_dot(do, v_buf[0, g], _NT), _dot(do, v_buf[1, g], _NT))
            p = p_all[head_tile(layer, g), :]
            ds = p * (dp - jnp.sum(dp * p, axis=-1, keepdims=True)) * scale
            dq = per_batch(_dot(ds, k_buf[0, g]), _dot(ds, k_buf[1, g]))
            do_all[head_tile(layer, g), :] = do
            ds_all[head_tile(layer, g), :] = ds
            dq_all[head_tile(layer, g), :] = dq
            acc = acc + _dot(spread_heads(dq), wq[:, head_cols(g)], _NT)
            dk_batch(t0 + 2 + g)
            return acc

        dxn = batch_sum(lax.fori_loop(0, hkv, head, jnp.zeros_like(dy)))
        return dy + _layernorm_bwd(dxn, att_xn[rows, :], att_rstd[rows, :1])

    for c in reads:
        c.wait()
    zero_fill(0, 0, lead)
    last_read.wait()

    out = lax.fori_loop(0, _LAYERS, forward, replicate(x_buf))
    out_buf[...] = compact(out).astype(out_buf.dtype)
    dx = lax.fori_loop(0, _LAYERS, backward, replicate(g_buf))
    dx_buf[...] = compact(dx).astype(dx_buf.dtype)

    def outer(dst, a, b):
        a_t = a.T.astype(_BF16)
        n = dst.shape[1]
        for i in range(dst.shape[0]):
            dst[i] = _dot(a_t[i * n:(i + 1) * n], b).astype(dst.dtype)

    dy_ffn = one_replica(ffn_dy[...])
    dh_ffn = one_replica(ffn_dh[...])
    db1[...] = jnp.sum(dh_ffn, axis=0).astype(db1.dtype)
    db2[...] = jnp.sum(dy_ffn, axis=0).astype(db2.dtype)
    outer(dw1, ffn_xn[...], dh_ffn)
    dv_batch(0)
    outer(dw2, _gelu(ffn_h[...]), dy_ffn)
    dv_batch(1)
    p_t[...] = p_all[...].T.astype(p_t.dtype)
    dv_batch(2)
    ds_t[...] = ds_all[...].T.astype(ds_t.dtype)
    att_xn_t[...] = att_xn[...].T.astype(att_xn_t.dtype)
    dv_batch(3)
    stack_row = lax.broadcasted_iota(jnp.int32, (_LAYERS * layer_rows, 1), 0)

    def both_layers(ref, g):
        return jnp.concatenate([ref[head_tile(l, g), :] for l in range(_LAYERS)], axis=0)

    def head_grads(g, carry):
        t0 = 4 + g * (nb + 1)
        for b in range(nb):
            mine = (stack_row % layer_rows) // rep == g * nb + b
            dk_buf[b, g] = _dot(ds_t[...], jnp.where(mine, q_all[...], 0.0)
                                ).astype(dk_buf.dtype)
            dv_buf[b, g] = _dot(p_t[...], jnp.where(mine, do_all[...], 0.0)
                                ).astype(dv_buf.dtype)
            dv_batch(t0 + b)
        dq = spread_heads(both_layers(dq_all, g))
        n = dwq.shape[1]
        for i in range(dwq.shape[0]):
            dwq[i, :, head_cols(g)] = _dot(att_xn_t[i * n:(i + 1) * n, :], dq
                                           ).astype(dwq.dtype)
        per_block = dwo.shape[1] // group_cols
        dwo[lax.div(g, per_block), head_cols(lax.rem(g, per_block)), :] = _dot(
            spread_heads(both_layers(o_all, g)).T, att_dy[...]).astype(dwo.dtype)
        dv_batch(t0 + nb)
        return carry

    lax.fori_loop(0, hkv, head_grads, 0)

    small = [pltpu.make_async_copy(s, d, out_sem.at[2]) for s, d in (
        (out_buf, out_hbm), (dx_buf, dx_hbm), (db1, db1_hbm), (db2, db2_hbm))]
    for c in small:
        c.start()

    def write_weights(*jobs):
        def body(i, carry):
            for src, dst, sem, cols in jobs:
                across = src.shape[2] // cols

                @pl.when(i < (src.shape[1] // _WEIGHT_ROWS) * across)
                def _():
                    r = pl.multiple_of(lax.div(i, across) * _WEIGHT_ROWS, _WEIGHT_ROWS)
                    c = pl.multiple_of(lax.rem(i, across) * cols, 128)
                    tile = (slice(None), pl.ds(r, _WEIGHT_ROWS), pl.ds(c, cols))
                    pltpu.make_async_copy(src.at[tile], dst.at[tile], sem).start()
            return carry

        for src, _, _, cols in jobs:
            assert src.shape[1] % _WEIGHT_ROWS == 0 and src.shape[2] % cols == 0
        steps = max((src.shape[1] // _WEIGHT_ROWS) * (src.shape[2] // cols)
                    for src, _, _, cols in jobs)
        lax.fori_loop(0, steps, body, 0)
        return [pltpu.make_async_copy(src, dst, sem) for src, dst, sem, _ in jobs]

    weights = (write_weights((dw1, dw1_hbm, out_sem.at[3], 256),
                             (dw2, dw2_hbm, out_sem.at[4], 256))
               + write_weights((dwq, dwq_hbm, out_sem.at[5], 256),
                               (dwo, dwo_hbm, out_sem.at[6], 256)))

    for which, src in enumerate((dk_buf, dv_buf)):
        for b in range(nb):
            def write_window(i, carry, which=which, src=src, b=b):
                r = pl.ds(pl.multiple_of(i * _WINDOW_ROWS, _WINDOW_ROWS), _WINDOW_ROWS)
                pltpu.make_async_copy(
                    src.at[b, :, r, :],
                    cache_grads[which].at[pl.ds(b * hkv, hkv), zero_segs, r, :],
                    out_sem.at[which]).start()
                return carry

            lax.fori_loop(0, win // _WINDOW_ROWS, write_window, 0)

    issued = (lead + 2 * _LAYERS * per_pass * batch, (4 + hkv * (nb + 1)) * batch)
    for which, done in enumerate(issued):
        assert done <= num_zero
        if done < num_zero:
            zero_fill(which, done, num_zero - done)

    for c in small + weights:
        c.wait()
    for which, ref in enumerate(cache_grads):
        pltpu.make_async_copy(ref, ref, out_sem.at[which]).wait()


@jax.jit
def pallas_interleave_layers__sliding_block_cached__dense_activation_gelu__decode_kernel(
    A_x: jax.Array,
    A_k_cache: jax.Array,
    A_v_cache: jax.Array,
    A_wq: jax.Array,
    A_wo: jax.Array,
    B_x: jax.Array,
    B_w1: jax.Array,
    B_b1: jax.Array,
    B_w2: jax.Array,
    B_b2: jax.Array,
    grad_out: jax.Array,
):
    del B_x
    nb, hkv, sk, dh = A_k_cache.shape
    d_model, d_ff = B_w1.shape
    win = min(4096, max(256, sk // 4))
    assert nb == 2 and _HQ == 4 * hkv and A_x.shape[1] == 1
    assert sk % win == 0 and win % _ZERO_ROWS == 0 and win % _WINDOW_ROWS == 0

    def vmem(a):
        return pltpu.VMEM(a.shape, a.dtype)

    def f32(*shape):
        return pltpu.VMEM(shape, _F32)

    def row_blocks(w, n):
        return jax.ShapeDtypeStruct((n, w.shape[0] // n, w.shape[1]), w.dtype)

    x = A_x.reshape(nb, d_model)
    g = grad_out.reshape(nb, d_model)
    d_cache = jax.ShapeDtypeStruct((nb * hkv, sk // win, win, dh), A_k_cache.dtype)
    d_wq, d_wo = row_blocks(A_wq, 4), row_blocks(A_wo, 4)
    d_w1, d_w2 = row_blocks(B_w1, 2), row_blocks(B_w2, 2)
    inputs = (x, A_k_cache, A_v_cache, A_wq, A_wo, B_w1, B_b1, B_w2, B_b2, g)
    outputs = (g, x, d_cache, d_cache, d_wq, d_wo, d_w1, B_b1, d_w2, B_b2)

    window = pltpu.VMEM((nb, hkv, win, dh), A_k_cache.dtype)
    heads = _LAYERS * hkv * 8
    layers = _LAYERS * 8
    hbm = pl.BlockSpec(memory_space=pl.ANY)
    out, dx, dk, dv, dwq, dwo, dw1, db1, dw2, db2 = pl.pallas_call(
        _kernel,
        out_shape=[jax.ShapeDtypeStruct(a.shape, a.dtype) for a in outputs],
        in_specs=[hbm] * len(inputs),
        out_specs=[hbm] * len(outputs),
        scratch_shapes=[
            window, window, vmem(A_wq), vmem(A_wo), vmem(B_w1), vmem(B_w2),
            vmem(x), vmem(g), vmem(B_b1), vmem(B_b2),
            pltpu.VMEM((sk // win - 1, _ZERO_ROWS, dh), A_k_cache.dtype),
            f32(heads, win), f32(heads, win),
            f32(heads, dh), f32(heads, dh), f32(heads, dh), f32(heads, dh),
            f32(layers, d_model), f32(layers, 128), f32(layers, d_model),
            f32(layers, d_model), f32(layers, 128), f32(layers, d_model),
            f32(layers, d_ff), f32(layers, d_ff),
            pltpu.VMEM((win, heads), _BF16), pltpu.VMEM((win, heads), _BF16),
            pltpu.VMEM((d_model, layers), _BF16),
            window, window, vmem(d_wq), vmem(d_wo), vmem(d_w1), vmem(d_w2),
            vmem(g), vmem(x), vmem(B_b1), vmem(B_b2),
            pltpu.SemaphoreType.DMA((2,)),
            pltpu.SemaphoreType.DMA((7,)),
        ],
        compiler_params=pltpu.CompilerParams(vmem_limit_bytes=110 * 1024 * 1024),
    )(*inputs)
    return (out.reshape(grad_out.shape), dx.reshape(A_x.shape),
            dk.reshape(A_k_cache.shape), dv.reshape(A_v_cache.shape),
            dwq.reshape(A_wq.shape), dwo.reshape(A_wo.shape),
            dw1.reshape(B_w1.shape), db1, dw2.reshape(B_w2.shape), db2)
```
